```python
import jax
import jax.numpy as jnp

def _softmax(x, axis=-1):
    return jax.nn.softmax(x, axis=axis)

def _gelu(x):
    return jax.nn.gelu(x, approximate=True)

def _silu(x):
    return jax.nn.silu(x)

def _sigmoid(x):
    return jax.nn.sigmoid(x)

def _layernorm(x, axis=-1, eps=1e-05):
    m = jnp.mean(x, axis=axis, keepdims=True)
    v = jnp.var(x, axis=axis, keepdims=True)
    return (x - m) / jnp.sqrt(v + eps)

def _scatter_add(tgt, idx, src, axis=0):
    return tgt.at[idx].add(src)

def _segment_sum(src, seg, n):
    return jax.ops.segment_sum(src, seg, n)

class _Rng:

    def __init__(self, key):
        self._k = key

    def _next(self):
        self._k, sub = jax.random.split(self._k)
        return sub

    def normal(self, shape):
        return jax.random.normal(self._next(), shape, dtype=jnp.bfloat16)

    def randint(self, lo, hi, shape):
        return jax.random.randint(self._next(), shape, lo, hi, dtype=jnp.int32)

    def uniform(self, shape, lo=0.0, hi=1.0):
        return jax.random.uniform(self._next(), shape, jnp.bfloat16, lo, hi)

    def permutation(self, n):
        return jax.random.permutation(self._next(), n)
kernel_name = 'adaLN_cond__sliding_block_cached__glu_gated_glu__decode'

def setup_inputs():
    _rng = _Rng(jax.random.key(int.from_bytes(__import__("os").urandom(4), "little")))
    _w = lambda a: (lambda t: t.astype(jnp.bfloat16) if jnp.issubdtype(t.dtype, jnp.floating) else t)(jnp.asarray(a))

    def _A_setup():
        B, Sq, D = (8, 1, 512)
        Hq, Hkv, Sk, Dh = (32, 32, 4096, 128)
        assert Hq % Hkv == 0, (Hq, Hkv)
        return {'x': _w((lambda *s: _rng.normal(s) * 0.05)(B, Sq, D)), 'k_cache': _w((lambda *s: _rng.normal(s) * 0.05)(B, Hkv, Sk, Dh)), 'v_cache': _w((lambda *s: _rng.normal(s) * 0.05)(B, Hkv, Sk, Dh)), 'wq': _w((lambda *s: _rng.normal(s) * 0.05)(D, Hq * Dh) * D ** (-0.5)), 'wo': _w((lambda *s: _rng.normal(s) * 0.05)(Hq * Dh, D) * (Hq * Dh) ** (-0.5))}
    _A_in = _A_setup()

    def _B_setup():
        B, S, D, F = (8, 1, 512, 1376)
        return {'x': _w((lambda *s: _rng.normal(s) * 0.05)(B, S, D)), 'w_gate': _w((lambda *s: _rng.normal(s) * 0.05)(D, F)), 'w_up': _w((lambda *s: _rng.normal(s) * 0.05)(D, F)), 'w_down': _w((lambda *s: _rng.normal(s) * 0.05)(F, D))}
    _B_in = _B_setup()
    return {'A_x': _A_in['x'], 'A_k_cache': _A_in['k_cache'], 'A_v_cache': _A_in['v_cache'], 'A_wq': _A_in['wq'], 'A_wo': _A_in['wo'], 'B_x': _B_in['x'], 'B_w_gate': _B_in['w_gate'], 'B_w_up': _B_in['w_up'], 'B_w_down': _B_in['w_down'], 'c': _w((lambda *s: _rng.normal(s) * 0.05)(8, 512)), 'w_mod': _w((lambda *s: _rng.normal(s) * 0.05)(512, 6 * 512) * 512 ** (-0.5))}

def reference(A_x, A_k_cache, A_v_cache, A_wq, A_wo, B_x, B_w_gate, B_w_up, B_w_down, c, w_mod):

    def _A_ref(x, k_cache, v_cache, wq, wo):
        B, Sq, D = x.shape
        Hq, Dh = (32, 128)
        Hkv, Sk = (k_cache.shape[1], k_cache.shape[2])
        W = min(4096, max(256, Sk // 4))
        rep = Hq // Hkv
        q = (lambda x, *d: x.transpose(*d))((x @ wq).reshape(B, Sq, Hq, Dh), 0, 2, 1, 3)
        k = jnp.repeat(k_cache[:, :, Sk - W:, :], rep, axis=1)
        v = jnp.repeat(v_cache[:, :, Sk - W:, :], rep, axis=1)
        scores = jnp.einsum('bhqd,bhkd->bhqk', q, k) * Dh ** (-0.5)
        p = _softmax(scores, axis=-1)
        o = jnp.einsum('bhqk,bhkd->bhqd', p, v)
        return (lambda x, *d: x.transpose(*d))(o, 0, 2, 1, 3).reshape(B, Sq, Hq * Dh) @ wo

    def _B_ref(x, w_gate, w_up, w_down):
        g = jnp.einsum('bsd,df->bsf', x, w_gate)
        u = jnp.einsum('bsd,df->bsf', x, w_up)
        h = _sigmoid(g) * u
        return jnp.einsum('bsf,fd->bsd', h, w_down)
    x = A_x
    mod = (_silu(c) @ w_mod).reshape(c.shape[0], 6, 1, -1)
    sa, ca, ga, sb, cb, gb = (mod[:, 0].copy(), mod[:, 1].copy(), mod[:, 2].copy(), mod[:, 3].copy(), mod[:, 4].copy(), mod[:, 5].copy())
    h = _layernorm(x, axis=-1) * (1 + ca) + sa
    x = x + ga * _A_ref(h, A_k_cache, A_v_cache, A_wq, A_wo)
    h = _layernorm(x, axis=-1) * (1 + cb) + sb
    x = x + gb * _B_ref(h, B_w_gate, B_w_up, B_w_down)
    return x
```

```python
import functools

import jax
import jax.numpy as jnp
from jax import lax
import jax.experimental.pallas as pl
import jax.experimental.pallas.tpu as pltpu

F32 = jnp.float32
BF16 = jnp.bfloat16


def _ln(x):
    m = jnp.mean(x, axis=-1, keepdims=True)
    xc = x - m
    v = jnp.mean(xc * xc, axis=-1, keepdims=True)
    return xc * lax.rsqrt(v + 1e-5)


def _mm(a, b):
    return jnp.dot(a, b, preferred_element_type=F32)


def _mm_t(a, b):
    return lax.dot_general(a, b, (((1,), (1,)), ((), ())), preferred_element_type=F32)


def make(rows=64, depth=8, late='end', nobc=False):
    def fn(A_x, A_k_cache, A_v_cache, A_wq, A_wo, B_x, B_w_gate, B_w_up, B_w_down, c, w_mod):
        del B_x
        B, _, D = A_x.shape
        _, H, S, DH = A_k_cache.shape
        F = B_w_gate.shape[1]
        W = min(4096, max(256, S // 4))
        NP = 2 * B
        nd = W // rows
        scale = DH ** -0.5

        def kern(x_hbm, c_hbm, k_hbm, v_hbm, wq_hbm, wo_hbm, wg_hbm, wu_hbm, wd_hbm, wm_hbm, out_hbm,
                 x_v, c_v, wm_v, wq_v, wo_v, wg_v, wu_v, wd_v, kv_v, q_v, acc_v, out_v, kv_sem, w_sem):

            def piece_start(h, p):
                src = k_hbm if p < B else v_hbm
                b = p % B
                for s in range(nd):
                    pltpu.make_async_copy(
                        src.at[b, h, pl.ds(S - W + s * rows, rows), :],
                        kv_v.at[p, pl.ds(s * rows, rows), :], kv_sem.at[p]).start(priority=s % 2)

            def piece_wait(p):
                pltpu.make_async_copy(kv_v.at[p], kv_v.at[p], kv_sem.at[p]).wait()

            def wcopy(src, dst, i):
                return pltpu.make_async_copy(src, dst, w_sem.at[i])

            cx = wcopy(x_hbm, x_v, 0)
            cc = wcopy(c_hbm, c_v, 1)
            cm = wcopy(wm_hbm, wm_v, 2)
            cq = wcopy(wq_hbm, wq_v, 3)
            co = wcopy(wo_hbm, wo_v, 4)
            cg = wcopy(wg_hbm, wg_v, 5)
            cu = wcopy(wu_hbm, wu_v, 6)
            cd = wcopy(wd_hbm, wd_v, 7)

            cc.start(); cx.start(); cm.start(); cq.start(priority=1)
            for p in range(depth):
                piece_start(0, p)

            cc.wait(); cx.wait(); cm.wait()
            cv = c_v[...].astype(F32)
            sc = (cv * jax.nn.sigmoid(cv)).astype(BF16)
            mod_a = _mm(sc, wm_v[:, 0:2 * D])
            x = x_v[...].astype(F32)
            h1 = (_ln(x) * (1.0 + mod_a[:, D:2 * D]) + mod_a[:, 0:D]).astype(BF16)
            cq.wait()
            q_v[...] = _mm(h1, wq_v[...]).astype(BF16)
            acc_v[...] = jnp.zeros_like(acc_v)
            row = lax.broadcasted_iota(jnp.int32, (B, W), 0)
            rowo = lax.broadcasted_iota(jnp.int32, (B, DH), 0)

            def head(h, issue):
                hs = pl.multiple_of(h * DH, DH)
                q = q_v[:, pl.ds(hs, DH)]
                s_all = None
                for b in range(B):
                    piece_wait(b)
                    issue(h, b)
                    s = _mm_t(q, kv_v[b])
                    s_all = s if s_all is None else jnp.where(row == b, s, s_all)
                m = jnp.max(s_all, axis=-1, keepdims=True)
                e = jnp.exp((s_all - m) * scale)
                l = jnp.sum(e, axis=-1, keepdims=True)
                pb = e.astype(BF16)
                o_all = None
                for b in range(B):
                    piece_wait(B + b)
                    issue(h, B + b)
                    o = _mm(pb, kv_v[B + b])
                    o_all = o if o_all is None else jnp.where(rowo == b, o, o_all)
                o = (o_all / l).astype(BF16)
                return o, hs

            def issue_loop(h, p):
                if p + depth < NP:
                    piece_start(h, p + depth)
                else:
                    piece_start(h + 1, p + depth - NP)

            if late != 'end':
                co.start(); cg.start(priority=1); cu.start(); cd.start(priority=1)
            else:
                co.start()
            co.wait()

            def body(h, carry):
                o, hs = head(h, issue_loop)
                acc_v[...] += _mm(o, wo_v[pl.ds(hs, DH), :])
                return carry

            lax.fori_loop(0, H - 1, body, 0)

            def issue_last(h, p):
                if p + depth < NP:
                    piece_start(h, p + depth)
                elif late == 'end':
                    j = p + depth - NP
                    if j == 0:
                        cg.start()
                    elif j == 1:
                        cu.start(priority=1)
                    elif j == 2:
                        cd.start()

            o, hs = head(H - 1, issue_last)
            attn = acc_v[...] + _mm(o, wo_v[pl.ds((H - 1) * DH, DH), :])
            mod_b = _mm(sc, wm_v[:, 2 * D:6 * D])
            ga, sb, cb, gb = (mod_b[:, i * D:(i + 1) * D] for i in range(4))
            x2 = x + ga * attn
            h2 = (_ln(x2) * (1.0 + cb) + sb).astype(BF16)
            cg.wait(); cu.wait()
            g = _mm_t(h2, wg_v[...])
            u = _mm_t(h2, wu_v[...])
            h3 = (jax.nn.sigmoid(g) * u).astype(BF16)
            cd.wait()
            y = x2 + gb * _mm(h3, wd_v[...])
            out_v[...] = y.astype(BF16)
            cout = pltpu.make_async_copy(out_v, out_hbm, w_sem.at[0])
            cout.start()
            cout.wait()

        hbm = pl.BlockSpec(memory_space=pltpu.HBM)
        out = pl.pallas_call(
            kern,
            out_shape=jax.ShapeDtypeStruct((B, D), BF16),
            in_specs=[hbm] * 10,
            out_specs=hbm,
            scratch_shapes=[
                pltpu.VMEM((B, D), BF16), pltpu.VMEM((B, D), BF16),
                pltpu.VMEM((D, 6 * D), BF16), pltpu.VMEM((D, H * DH), BF16), pltpu.VMEM((H * DH, D), BF16),
                pltpu.VMEM((F, D), BF16), pltpu.VMEM((F, D), BF16), pltpu.VMEM((F, D), BF16),
                pltpu.VMEM((NP, W, DH), BF16), pltpu.VMEM((B, H * DH), BF16), pltpu.VMEM((B, D), F32),
                pltpu.VMEM((B, D), BF16),
                pltpu.SemaphoreType.DMA((NP,)), pltpu.SemaphoreType.DMA((8,)),
            ],
            compiler_params=pltpu.CompilerParams(vmem_limit_bytes=100 * 1024 * 1024, disable_bounds_checks=nobc),
        )(A_x.reshape(B, D), c, A_k_cache, A_v_cache, A_wq, A_wo, B_w_gate.T, B_w_up.T, B_w_down, w_mod)
        return out.reshape(B, 1, D)
    return fn


@jax.jit
def pallas_adaLN_cond__sliding_block_cached__glu_gated_glu__decode_kernel(
    A_x, A_k_cache, A_v_cache, A_wq, A_wo, B_x, B_w_gate, B_w_up, B_w_down, c, w_mod):
    return make()(A_x, A_k_cache, A_v_cache, A_wq, A_wo, B_x, B_w_gate, B_w_up, B_w_down, c, w_mod)
```

```python
import functools

import jax
import jax.numpy as jnp
from jax import lax
import jax.experimental.pallas as pl
import jax.experimental.pallas.tpu as pltpu

F32 = jnp.float32
BF16 = jnp.bfloat16
T = 128


def _ln(x):
    m = jnp.mean(x, axis=-1, keepdims=True)
    xc = x - m
    v = jnp.mean(xc * xc, axis=-1, keepdims=True)
    return xc * lax.rsqrt(v + 1e-5)


def _mm(a, b):
    return jnp.dot(a, b, preferred_element_type=F32)


def _mm_t(a, b):
    return lax.dot_general(a, b, (((1,), (1,)), ((), ())), preferred_element_type=F32)


def make(depth=12, stag=1, order='kkvv', border=None, nobc=False, where='post'):
    def fn(A_x, A_k_cache, A_v_cache, A_wq, A_wo, B_x, B_w_gate, B_w_up, B_w_down, c, w_mod):
        del B_x
        B, _, D = A_x.shape
        _, H, S, DH = A_k_cache.shape
        F = B_w_gate.shape[1]
        W = min(4096, max(256, S // 4))
        NK = W // T
        NG = 2 * NK
        scale = DH ** -0.5
        r0 = F % T
        fch = ([(0, r0)] if r0 else []) + [(r0 + i * T, T) for i in range(F // T)]
        NF = len(fch)
        bord = list(border) if border is not None else list(range(B))
        if order == 'kkvv':
            seq = list(range(NG))
        else:
            seq = [g for kb in range(NK) for g in (kb, NK + kb)]
        pos = {g: i for i, g in enumerate(seq)}

        def kern(x_hbm, c_hbm, k_hbm, v_hbm, wq_hbm, wo_hbm, wg_hbm, wu_hbm, wd_hbm, wm_hbm, out_hbm,
                 x_v, c_v, wm_v, wq_v, wo_v, wg_v, wu_v, wd_v, kv_v, q_v, o_v, out_v,
                 kv_sem, s_sem, q_sem, gu_sem, d_sem):
            cp = pltpu.make_async_copy

            def wait(dst, sem):
                cp(dst, dst, sem).wait()

            def group_start(h, g):
                src = k_hbm if g < NK else v_hbm
                for i, b in enumerate(bord):
                    kb = (g + stag * b) % NK
                    cp(src.at[b, h, pl.ds(S - W + kb * T, T), :], kv_v.at[g, b], kv_sem.at[g]).start(priority=i % 2)

            def wq_start(j):
                for i in range(32):
                    sl = (pl.ds(128 * j + 8 * (i // 2), 8), pl.ds((i % 2) * 2048, 2048))
                    cp(wq_hbm.at[sl], wq_v.at[sl], q_sem.at[j]).start(priority=i % 2)

            def side_start(h):
                for i in range(4):
                    sl = pl.ds(pl.multiple_of(h * DH + 32 * i, 32), 32)
                    cp(wo_hbm.at[sl], wo_v.at[sl], s_sem.at[3]).start(priority=i % 2)
                for i in range(2):
                    sl = (pl.ds(pl.multiple_of(h * 16 + 8 * i, 8), 8), pl.ds(2 * D, 4 * D))
                    cp(wm_hbm.at[sl], wm_v.at[sl], s_sem.at[4]).start(priority=i % 2)

            late = []
            for j, (r, n) in enumerate(fch):
                for i in range(n // 32):
                    sl = pl.ds(r + 32 * i, 32)
                    late.append((wg_hbm, wg_v, sl, gu_sem, j))
                    late.append((wu_hbm, wu_v, sl, gu_sem, j))
            for j, (r, n) in enumerate(fch):
                for i in range(n // 32):
                    late.append((wd_hbm, wd_v, pl.ds(r + 32 * i, 32), d_sem, j))

            def late_start(lo, hi):
                for i in range(lo, min(hi, len(late))):
                    s_, d_, sl, sem, j = late[i]
                    cp(s_.at[sl], d_.at[sl], sem.at[j]).start(priority=i % 2)

            cp(c_hbm, c_v, s_sem.at[0]).start(priority=0)
            cp(x_hbm, x_v, s_sem.at[1]).start(priority=1)
            for i in range(32):
                sl = (pl.ds(16 * i, 16), pl.ds(0, 2 * D))
                cp(wm_hbm.at[sl], wm_v.at[sl], s_sem.at[2]).start(priority=i % 2)
            for j in range(3):
                wq_start(j)
            wait(c_v, s_sem.at[0])
            wait(x_v, s_sem.at[1])
            wait(wm_v.at[:, pl.ds(0, 2 * D)], s_sem.at[2])
            wq_start(3)
            cv = c_v[...].astype(F32)
            sc = (cv * jax.nn.sigmoid(cv)).astype(BF16)
            mod_a = _mm(sc, wm_v[:, 0:2 * D])
            x = x_v[...].astype(F32)
            h1 = (_ln(x) * (1.0 + mod_a[:, D:2 * D]) + mod_a[:, 0:D]).astype(BF16)
            q = None
            for j in range(4):
                wait(wq_v.at[pl.ds(128 * j, 128)], q_sem.at[j])
                for p in range(j * depth // 4, (j + 1) * depth // 4):
                    group_start(0, seq[p])
                part = _mm(h1[:, 128 * j:128 * (j + 1)], wq_v[pl.ds(128 * j, 128), :])
                q = part if q is None else q + part
            q = q.astype(BF16)
            for h in range(H):
                q_v[h] = q[:, h * DH:(h + 1) * DH]

            row = lax.broadcasted_iota(jnp.int32, (B, DH), 0)

            def pick(xs):
                r = xs[0]
                for b in range(1, B):
                    r = jnp.where(row == b, xs[b], r)
                return r

            def head(h, issue):
                q = q_v[h]
                ss = []
                step = [0]

                def advance():
                    issue(h, step[0])
                    step[0] += 1

                for g in range(NK):
                    wait(kv_v.at[g], kv_sem.at[g])
                    if where == 'pre': advance()
                    ss.append(pick([_mm_t(q, kv_v[g, b]) for b in range(B)]))
                    if where == 'post': advance()
                m = ss[0]
                for s in ss[1:]:
                    m = jnp.maximum(m, s)
                m = jnp.max(m, axis=-1, keepdims=True)
                es = [jnp.exp((s - m) * scale) for s in ss]
                l = es[0]
                for e in es[1:]:
                    l = l + e
                l = jnp.sum(l, axis=-1, keepdims=True)
                o = None
                for g in range(NK):
                    wait(kv_v.at[NK + g], kv_sem.at[NK + g])
                    if where == 'pre': advance()
                    p = es[g].astype(BF16)
                    og = pick([_mm(p, kv_v[NK + g, b]) for b in range(B)])
                    o = og if o is None else o + og
                    if where == 'post': advance()
                o_v[h] = (o / l).astype(BF16)

            def issue_loop(h, p):
                if p == 0:
                    side_start(h)
                if p + depth < NG:
                    group_start(h, seq[p + depth])
                else:
                    group_start(h + 1, seq[p + depth - NG])

            def body(h, carry):
                head(h, issue_loop)
                return carry

            lax.fori_loop(0, H - 1, body, 0)

            nl = len(late)

            def issue_last(h, p):
                if p == 0:
                    side_start(h)
                if p + depth < NG:
                    group_start(h, seq[p + depth])
                else:
                    j = p + depth - NG
                    lo = (j * nl // depth + 1) // 2 * 2
                    hi = ((j + 1) * nl // depth + 1) // 2 * 2
                    late_start(lo, hi)

            head(H - 1, issue_last)

            wait(wo_v, s_sem.at[3])
            attn = None
            for h in range(H):
                part = _mm(o_v[h], wo_v[pl.ds(h * DH, DH), :])
                attn = part if attn is None else attn + part
            wait(wm_v.at[:, pl.ds(2 * D, 4 * D)], s_sem.at[4])
            mod_b = _mm(sc, wm_v[:, 2 * D:6 * D])
            ga, sb, cb, gb = (mod_b[:, i * D:(i + 1) * D] for i in range(4))
            x2 = x + ga * attn
            h2 = (_ln(x2) * (1.0 + cb) + sb).astype(BF16)
            h3 = []
            for j, (r, n) in enumerate(fch):
                wait(wg_v.at[pl.ds(0, 2 * n)], gu_sem.at[j])
                g = _mm_t(h2, wg_v[pl.ds(r, n), :])
                u = _mm_t(h2, wu_v[pl.ds(r, n), :])
                h3.append((jax.nn.sigmoid(g) * u).astype(BF16))
            y = None
            for j, (r, n) in enumerate(fch):
                wait(wd_v.at[pl.ds(r, n)], d_sem.at[j])
                part = _mm(h3[j], wd_v[pl.ds(r, n), :])
                y = part if y is None else y + part
            out_v[...] = (x2 + gb * y).astype(BF16)
            cout = cp(out_v, out_hbm, s_sem.at[0])
            cout.start()
            cout.wait()

        hbm = pl.BlockSpec(memory_space=pltpu.HBM)
        out = pl.pallas_call(
            kern,
            out_shape=jax.ShapeDtypeStruct((B, D), BF16),
            in_specs=[hbm] * 10,
            out_specs=hbm,
            scratch_shapes=[
                pltpu.VMEM((B, D), BF16), pltpu.VMEM((B, D), BF16),
                pltpu.VMEM((D, 6 * D), BF16), pltpu.VMEM((D, H * DH), BF16), pltpu.VMEM((H * DH, D), BF16),
                pltpu.VMEM((F, D), BF16), pltpu.VMEM((F, D), BF16), pltpu.VMEM((F, D), BF16),
                pltpu.VMEM((NG, B, T, DH), BF16), pltpu.VMEM((H, B, DH), BF16), pltpu.VMEM((H, B, DH), BF16),
                pltpu.VMEM((B, D), BF16),
                pltpu.SemaphoreType.DMA((NG,)), pltpu.SemaphoreType.DMA((5,)), pltpu.SemaphoreType.DMA((4,)),
                pltpu.SemaphoreType.DMA((NF,)), pltpu.SemaphoreType.DMA((NF,)),
            ],
            compiler_params=pltpu.CompilerParams(vmem_limit_bytes=100 * 1024 * 1024, disable_bounds_checks=nobc),
        )(A_x.reshape(B, D), c, A_k_cache, A_v_cache, A_wq, A_wo, B_w_gate.T, B_w_up.T, B_w_down, w_mod)
        return out.reshape(B, 1, D)
    return fn


@jax.jit
def pallas_adaLN_cond__sliding_block_cached__glu_gated_glu__decode_kernel(
    A_x, A_k_cache, A_v_cache, A_wq, A_wo, B_x, B_w_gate, B_w_up, B_w_down, c, w_mod):
    return make()(A_x, A_k_cache, A_v_cache, A_wq, A_wo, B_x, B_w_gate, B_w_up, B_w_down, c, w_mod)
```

```python
import jax
import jax.numpy as jnp
from jax import lax
import jax.experimental.pallas as pl
import jax.experimental.pallas.tpu as pltpu

F32 = jnp.float32
BF16 = jnp.bfloat16

T = 128
DEPTH = 12
STAG = 6
K_SHIFT = 64
ROWS = 32


def _layernorm(x):
    m = jnp.mean(x, axis=-1, keepdims=True)
    xc = x - m
    v = jnp.mean(xc * xc, axis=-1, keepdims=True)
    return xc * lax.rsqrt(v + 1e-5)


def _mm(a, b):
    return jnp.dot(a, b, preferred_element_type=F32)


def _mm_t(a, b):
    return lax.dot_general(a, b, (((1,), (1,)), ((), ())), preferred_element_type=F32)


def _kernel(x_hbm, c_hbm, k_hbm, v_hbm, wq_hbm, wo_hbm, wg_hbm, wu_hbm, wd_hbm, wm_hbm, out_hbm,
            x_v, c_v, wm_v, wq_v, wo_v, wg_v, wu_v, wd_v, kv_v, q_v, o_v, out_v, sems):
    B, H, S, DH = k_hbm.shape
    F, D = wg_hbm.shape
    W = min(4096, max(256, S // 4))
    NK = W // T
    NG = 2 * NK
    NB = D // DH
    fch = [(r, min(T, F - r)) for r in range(0, F, T)]
    NF = len(fch)
    scale = DH ** -0.5

    kv_sem = lambda g: sems.at[g]
    c_sem, x_sem, wa_sem, wo_sem, wb_sem = (sems.at[NG + i] for i in range(5))
    q_sem = lambda j: sems.at[NG + 5 + j]
    gu_sem = lambda j: sems.at[NG + 5 + NB + j]
    d_sem = lambda j: sems.at[NG + 5 + NB + NF + j]

    queue = [0]

    def start(src, dst, sem):
        pltpu.make_async_copy(src, dst, sem).start(priority=queue[0])
        queue[0] ^= 1

    def wait(dst, sem):
        pltpu.make_async_copy(dst, dst, sem).wait()

    def start_group(h, g):
        src, shift = (k_hbm, K_SHIFT) if g < NK else (v_hbm, 0)
        for b in range(B):
            r = (g + STAG * b) % NK * T + shift
            n = min(T, W - r)
            start(src.at[b, h, pl.ds(S - W + r, n)], kv_v.at[g, b, pl.ds(0, n)], kv_sem(g))
            if n < T:
                start(src.at[b, h, pl.ds(S - W, T - n)], kv_v.at[g, b, pl.ds(n, T - n)], kv_sem(g))

    def start_wq(j):
        for i in range(8):
            for c0, n in ((0, 1024), (1024, 2048), (3072, 1024)):
                for half in range(2):
                    sl = (pl.ds(DH * j + 64 * half + 8 * i, 8), pl.ds(c0, n))
                    start(wq_hbm.at[sl], wq_v.at[sl], q_sem(j))

    def start_side(h):
        n = H * DH // ROWS // H
        for i in range(n):
            sl = pl.ds(pl.multiple_of((h + H * i) * ROWS, ROWS), ROWS)
            start(wo_hbm.at[sl], wo_v.at[sl], wo_sem)
        for i in range(D // 8 // H):
            sl = (pl.ds(pl.multiple_of((h + H * i) * 8, 8), 8), pl.ds(2 * D, 4 * D))
            start(wm_hbm.at[sl], wm_v.at[sl], wb_sem)

    late = []
    for j, (r, n) in enumerate(fch):
        for i in range(0, n, ROWS):
            late.append((wg_hbm, wg_v, pl.ds(r + i, ROWS), gu_sem(j)))
            late.append((wu_hbm, wu_v, pl.ds(r + i, ROWS), gu_sem(j)))
    for j, (r, n) in enumerate(fch):
        for i in range(0, n, ROWS):
            late.append((wd_hbm, wd_v, pl.ds(r + i, ROWS), d_sem(j)))

    start(c_hbm, c_v, c_sem)
    start(x_hbm, x_v, x_sem)
    for r in range(0, D, 16):
        sl = (pl.ds(r, 16), pl.ds(0, 2 * D))
        start(wm_hbm.at[sl], wm_v.at[sl], wa_sem)
    for j in range(NB - 1):
        start_wq(j)
    wait(c_v, c_sem)
    wait(x_v, x_sem)
    wait(wm_v.at[:, pl.ds(0, 2 * D)], wa_sem)
    start_wq(NB - 1)

    cv = c_v[...].astype(F32)
    silu_c = (cv * jax.nn.sigmoid(cv)).astype(BF16)
    mod_a = _mm(silu_c, wm_v[:, 0:2 * D])
    x = x_v[...].astype(F32)
    h1 = (_layernorm(x) * (1.0 + mod_a[:, D:2 * D]) + mod_a[:, 0:D]).astype(BF16)
    q = None
    for j in range(NB):
        wait(wq_v.at[pl.ds(DH * j, DH)], q_sem(j))
        for g in range(j * DEPTH // NB, (j + 1) * DEPTH // NB):
            start_group(0, g)
        part = _mm(h1[:, DH * j:DH * (j + 1)], wq_v[pl.ds(DH * j, DH), :])
        q = part if q is None else q + part
    q = q.astype(BF16)
    for h in range(H):
        q_v[h] = q[:, h * DH:(h + 1) * DH]

    row = lax.broadcasted_iota(jnp.int32, (B, DH), 0)
    lane = lax.broadcasted_iota(jnp.int32, (B, T), 1)

    def own_rows(xs):
        r = xs[0]
        for b in range(1, B):
            r = jnp.where(row == b, xs[b], r)
        return r

    def head(h, issue):
        qh = q_v[h]
        s = []
        for g in range(NK):
            wait(kv_v.at[g], kv_sem(g))
            s.append(own_rows([_mm_t(qh, kv_v[g, b]) for b in range(B)]))
            issue(h, g)
        m = s[0]
        for t in s[1:]:
            m = jnp.maximum(m, t)
        m = jnp.max(m, axis=-1, keepdims=True)
        e = [jnp.exp((t - m) * scale) for t in s]
        l = e[0]
        for t in e[1:]:
            l = l + t
        l = jnp.sum(l, axis=-1, keepdims=True)
        if K_SHIFT:
            e = [pltpu.roll(t, K_SHIFT, 1) for t in e]
            e = [jnp.where(lane < K_SHIFT, e[g - 1], e[g]) for g in range(NK)]
        o = None
        for g in range(NK):
            wait(kv_v.at[NK + g], kv_sem(NK + g))
            p = e[g].astype(BF16)
            og = own_rows([_mm(p, kv_v[NK + g, b]) for b in range(B)])
            o = og if o is None else o + og
            issue(h, NK + g)
        o_v[h] = (o / l).astype(BF16)

    def issue_steady(h, g):
        if g == 0:
            start_side(h)
        if g + DEPTH < NG:
            start_group(h, g + DEPTH)
        else:
            start_group(h + 1, g + DEPTH - NG)

    def issue_last(h, g):
        if g == 0:
            start_side(h)
        if g + DEPTH < NG:
            start_group(h, g + DEPTH)
        else:
            j = g + DEPTH - NG
            lo, hi = (2 * ((i * len(late) // DEPTH + 1) // 2) for i in (j, j + 1))
            for src, dst, sl, sem in late[lo:hi]:
                start(src.at[sl], dst.at[sl], sem)

    def body(h, carry):
        head(h, issue_steady)
        return carry

    lax.fori_loop(0, H - 1, body, 0)
    head(H - 1, issue_last)

    wait(wo_v, wo_sem)
    attn = None
    for h in range(H):
        part = _mm(o_v[h], wo_v[pl.ds(h * DH, DH), :])
        attn = part if attn is None else attn + part
    wait(wm_v.at[:, pl.ds(2 * D, 4 * D)], wb_sem)
    mod_b = _mm(silu_c, wm_v[:, 2 * D:6 * D])
    ga, sb, cb, gb = (mod_b[:, i * D:(i + 1) * D] for i in range(4))
    x2 = x + ga * attn
    h2 = (_layernorm(x2) * (1.0 + cb) + sb).astype(BF16)
    h3 = []
    for j, (r, n) in enumerate(fch):
        wait(wg_v.at[pl.ds(r, n)], gu_sem(j))
        wait(wu_v.at[pl.ds(r, n)], gu_sem(j))
        g = _mm_t(h2, wg_v[pl.ds(r, n), :])
        u = _mm_t(h2, wu_v[pl.ds(r, n), :])
        h3.append((jax.nn.sigmoid(g) * u).astype(BF16))
    y = None
    for j, (r, n) in enumerate(fch):
        wait(wd_v.at[pl.ds(r, n)], d_sem(j))
        part = _mm(h3[j], wd_v[pl.ds(r, n), :])
        y = part if y is None else y + part
    out_v[...] = (x2 + gb * y).astype(BF16)
    done = pltpu.make_async_copy(out_v, out_hbm, c_sem)
    done.start()
    done.wait()


@jax.jit
def pallas_adaLN_cond__sliding_block_cached__glu_gated_glu__decode_kernel(
    A_x: jax.Array,
    A_k_cache: jax.Array,
    A_v_cache: jax.Array,
    A_wq: jax.Array,
    A_wo: jax.Array,
    B_x: jax.Array,
    B_w_gate: jax.Array,
    B_w_up: jax.Array,
    B_w_down: jax.Array,
    c: jax.Array,
    w_mod: jax.Array,
):
    del B_x
    B, _, D = A_x.shape
    _, H, S, DH = A_k_cache.shape
    F = B_w_gate.shape[1]
    W = min(4096, max(256, S // 4))
    NG = 2 * (W // T)
    NF = -(-F // T)
    assert (B, H, DH, D) == (8, 32, 128, 512) and W % T == 0 and F % ROWS == 0 and DEPTH <= NG

    hbm = pl.BlockSpec(memory_space=pltpu.HBM)
    out = pl.pallas_call(
        _kernel,
        out_shape=jax.ShapeDtypeStruct((B, D), BF16),
        in_specs=[hbm] * 10,
        out_specs=hbm,
        scratch_shapes=[
            pltpu.VMEM((B, D), BF16),
            pltpu.VMEM((B, D), BF16),
            pltpu.VMEM((D, 6 * D), BF16),
            pltpu.VMEM((D, H * DH), BF16),
            pltpu.VMEM((H * DH, D), BF16),
            pltpu.VMEM((F, D), BF16),
            pltpu.VMEM((F, D), BF16),
            pltpu.VMEM((F, D), BF16),
            pltpu.VMEM((NG, B, T, DH), BF16),
            pltpu.VMEM((H, B, DH), BF16),
            pltpu.VMEM((H, B, DH), BF16),
            pltpu.VMEM((B, D), BF16),
            pltpu.SemaphoreType.DMA((NG + 5 + D // DH + 2 * NF,)),
        ],
        compiler_params=pltpu.CompilerParams(
            vmem_limit_bytes=64 * 1024 * 1024,
            disable_semaphore_checks=True,
        ),
    )(A_x.reshape(B, D), c, A_k_cache, A_v_cache, A_wq, A_wo,
      B_w_gate.T, B_w_up.T, B_w_down, w_mod)
    return out.reshape(B, 1, D)
```

```python
import jax
import jax.numpy as jnp
from jax import lax
import jax.experimental.pallas as pl
import jax.experimental.pallas.tpu as pltpu

F32 = jnp.float32
BF16 = jnp.bfloat16

T = 128
DEPTH = 12
STAG = 6
K_SHIFT = 64
ROWS = 32
GU_CHUNKS = (384, 384, 384, 224)
D_CHUNKS = (384, 384, 256, 352)
EPI = (8, 8, 8, 9)


def _chunks(sizes):
    out, r = [], 0
    for n in sizes:
        out.append((r, n))
        r += n
    return out


def _layernorm(x):
    m = jnp.mean(x, axis=-1, keepdims=True)
    xc = x - m
    v = jnp.mean(xc * xc, axis=-1, keepdims=True)
    return xc * lax.rsqrt(v + 1e-5)


def _mm(a, b):
    return jnp.dot(a, b, preferred_element_type=F32)


def _mm_t(a, b):
    return lax.dot_general(a, b, (((1,), (1,)), ((), ())), preferred_element_type=F32)


def _kernel(x_hbm, c_hbm, k_hbm, v_hbm, wq_hbm, wo_hbm, wg_hbm, wu_hbm, wd_hbm, wm_hbm, out_hbm,
            x_v, c_v, wm_v, wq_v, wo_v, wg_v, wu_v, wd_v, kv_v, q_v, acc_v, mod_v, out_v, sems):
    B, H, S, DH = k_hbm.shape
    F, D = wg_hbm.shape
    W = min(4096, max(256, S // 4))
    NK = W // T
    NG = 2 * NK
    NB = D // DH
    gu_ch, d_ch = _chunks(GU_CHUNKS), _chunks(D_CHUNKS)
    scale = DH ** -0.5

    kv_sem = lambda g: sems.at[g]
    c_sem, x_sem, wa_sem, wo_sem, wb_sem = (sems.at[NG + i] for i in range(5))
    q_sem = lambda j: sems.at[NG + 5 + j]
    gu_sem = lambda j: sems.at[NG + 5 + NB + j]
    d_sem = lambda j: sems.at[NG + 5 + NB + len(gu_ch) + j]

    queue = [0]

    def start(src, dst, sem):
        pltpu.make_async_copy(src, dst, sem).start(priority=queue[0])
        queue[0] ^= 1

    def start_list(copies):
        for src, dst, sl, sem in copies:
            start(src.at[sl], dst.at[sl], sem)

    def wait(dst, sem):
        pltpu.make_async_copy(dst, dst, sem).wait()

    def start_group(h, g):
        src, shift = (k_hbm, K_SHIFT) if g < NK else (v_hbm, 0)
        for b in range(B):
            r = (g + 1 + STAG * b) % NK * T + shift
            n = min(T, W - r)
            start(src.at[b, h, pl.ds(S - W + r, n)], kv_v.at[g, b, pl.ds(0, n)], kv_sem(g))
            if n < T:
                start(src.at[b, h, pl.ds(S - W, T - n)], kv_v.at[g, b, pl.ds(n, T - n)], kv_sem(g))

    def start_wq(j):
        for i in range(8):
            for c0, n in ((0, 1024), (1024, 2048), (3072, 1024)):
                for half in range(2):
                    sl = (pl.ds(DH * j + 64 * half + 8 * i, 8), pl.ds(c0, n))
                    start(wq_hbm.at[sl], wq_v.at[sl], q_sem(j))

    wo_c = [(wo_hbm, wo_v, pl.ds(r + k * H * DH // 4, ROWS), wo_sem)
            for r in range(0, H * DH // 4, ROWS) for k in range(4)]
    wb_c = [(wm_hbm, wm_v, (pl.ds(r + k * D // 2, 8), pl.ds(2 * D, 4 * D)), wb_sem)
            for r in range(0, D // 2, 8) for k in range(2)]
    side = []
    for i in range(len(wb_c)):
        side += [wo_c[2 * i], wb_c[i], wo_c[2 * i + 1]]
    per = len(side) // NB

    late = []
    for j, (r, n) in enumerate(gu_ch):
        for i in range(0, n, ROWS):
            late.append((wg_hbm, wg_v, pl.ds(r + i, ROWS), gu_sem(j)))
            late.append((wu_hbm, wu_v, pl.ds(r + i, ROWS), gu_sem(j)))
    for j, (r, n) in enumerate(d_ch):
        for i in range(0, n, ROWS):
            late.append((wd_hbm, wd_v, pl.ds(r + i, ROWS), d_sem(j)))

    start(c_hbm, c_v, c_sem)
    start(x_hbm, x_v, x_sem)
    for r in range(0, D, 16):
        sl = (pl.ds(r, 16), pl.ds(0, 2 * D))
        start(wm_hbm.at[sl], wm_v.at[sl], wa_sem)
    for j in range(NB - 1):
        start_wq(j)
    wait(c_v, c_sem)
    wait(x_v, x_sem)
    wait(wm_v.at[:, pl.ds(0, 2 * D)], wa_sem)
    start_wq(NB - 1)

    cv = c_v[...].astype(F32)
    silu_c = (cv * jax.nn.sigmoid(cv)).astype(BF16)
    mod_a = _mm(silu_c, wm_v[:, 0:2 * D])
    x = x_v[...].astype(F32)
    h1 = (_layernorm(x) * (1.0 + mod_a[:, D:2 * D]) + mod_a[:, 0:D]).astype(BF16)
    q = None
    for j in range(NB):
        wait(wq_v.at[pl.ds(DH * j, DH)], q_sem(j))
        start_list(side[j * per:(j + 1) * per])
        part = _mm(h1[:, DH * j:DH * (j + 1)], wq_v[pl.ds(DH * j, DH), :])
        q = part if q is None else q + part
    q = q.astype(BF16)
    for h in range(H):
        q_v[h] = q[:, h * DH:(h + 1) * DH]
    for g in range(DEPTH // 2):
        start_group(0, g)
    wait(wm_v.at[:, pl.ds(2 * D, 4 * D)], wb_sem)
    wait(wo_v, wo_sem)
    for g in range(DEPTH // 2, DEPTH):
        start_group(0, g)
    mod_v[...] = _mm(silu_c, wm_v[:, 2 * D:6 * D])
    acc_v[...] = jnp.zeros_like(acc_v)

    row = lax.broadcasted_iota(jnp.int32, (B, DH), 0)
    lane = lax.broadcasted_iota(jnp.int32, (B, T), 1)

    def own_rows(xs):
        r = xs[0]
        for b in range(1, B):
            r = jnp.where(row == b, xs[b], r)
        return r

    def head(h, issue):
        qh = q_v[h]
        s = []
        for g in range(NK):
            wait(kv_v.at[g], kv_sem(g))
            s.append(own_rows([_mm_t(qh, kv_v[g, b]) for b in range(B)]))
            issue(h, g)
        m = s[0]
        for t in s[1:]:
            m = jnp.maximum(m, t)
        m = jnp.max(m, axis=-1, keepdims=True)
        e = [jnp.exp((t - m) * scale) for t in s]
        l = e[0]
        for t in e[1:]:
            l = l + t
        l = jnp.sum(l, axis=-1, keepdims=True)
        if K_SHIFT:
            e = [pltpu.roll(t, K_SHIFT, 1) for t in e]
            e = [jnp.where(lane < K_SHIFT, e[g - 1], e[g]) for g in range(NK)]
        o = None
        for g in range(NK):
            wait(kv_v.at[NK + g], kv_sem(NK + g))
            p = e[g].astype(BF16)
            og = own_rows([_mm(p, kv_v[NK + g, b]) for b in range(B)])
            o = og if o is None else o + og
            issue(h, NK + g)
        acc_v[...] += _mm((o / l).astype(BF16), wo_v[pl.ds(pl.multiple_of(h * DH, DH), DH), :])

    def issue_steady(h, g):
        if g + DEPTH < NG:
            start_group(h, g + DEPTH)
        else:
            start_group(h + 1, g + DEPTH - NG)

    def issue_last(h, g):
        if g + DEPTH < NG:
            start_group(h, g + DEPTH)
        else:
            j = g + DEPTH - NG
            start_list(late[j * B:(j + 1) * B])

    def body(h, carry):
        head(h, issue_steady)
        return carry

    lax.fori_loop(0, H - 1, body, 0)
    head(H - 1, issue_last)

    rest = late[DEPTH * B:]
    pos = [0]

    def more(k):
        n = EPI[k] if k < len(EPI) else len(rest)
        start_list(rest[pos[0]:pos[0] + n])
        pos[0] += n

    ga, sb, cb, gb = (mod_v[:, i * D:(i + 1) * D] for i in range(4))
    more(0)
    x2 = x + ga * acc_v[...]
    h2 = (_layernorm(x2) * (1.0 + cb) + sb).astype(BF16)
    h3 = []
    for j, (r, n) in enumerate(gu_ch):
        wait(wg_v.at[pl.ds(r, n)], gu_sem(j))
        wait(wu_v.at[pl.ds(r, n)], gu_sem(j))
        more(j + 1)
        g = _mm_t(h2, wg_v[pl.ds(r, n), :])
        u = _mm_t(h2, wu_v[pl.ds(r, n), :])
        h3.append((jax.nn.sigmoid(g) * u).astype(BF16))
    more(len(EPI))
    h3 = jnp.concatenate(h3, axis=1)
    y = None
    for j, (r, n) in enumerate(d_ch):
        wait(wd_v.at[pl.ds(r, n)], d_sem(j))
        part = _mm(h3[:, r:r + n], wd_v[pl.ds(r, n), :])
        y = part if y is None else y + part
    out_v[...] = (x2 + gb * y).astype(BF16)
    done = pltpu.make_async_copy(out_v, out_hbm, c_sem)
    done.start()
    done.wait()


@jax.jit
def pallas_adaLN_cond__sliding_block_cached__glu_gated_glu__decode_kernel(
    A_x: jax.Array,
    A_k_cache: jax.Array,
    A_v_cache: jax.Array,
    A_wq: jax.Array,
    A_wo: jax.Array,
    B_x: jax.Array,
    B_w_gate: jax.Array,
    B_w_up: jax.Array,
    B_w_down: jax.Array,
    c: jax.Array,
    w_mod: jax.Array,
):
    del B_x
    B, _, D = A_x.shape
    _, H, S, DH = A_k_cache.shape
    F = B_w_gate.shape[1]
    W = min(4096, max(256, S // 4))
    NG = 2 * (W // T)
    assert (B, H, DH, D) == (8, 32, 128, 512) and W % T == 0 and F % ROWS == 0
    assert DEPTH <= NG and sum(GU_CHUNKS) == F == sum(D_CHUNKS)

    hbm = pl.BlockSpec(memory_space=pltpu.HBM)
    out = pl.pallas_call(
        _kernel,
        out_shape=jax.ShapeDtypeStruct((B, D), BF16),
        in_specs=[hbm] * 10,
        out_specs=hbm,
        scratch_shapes=[
            pltpu.VMEM((B, D), BF16),
            pltpu.VMEM((B, D), BF16),
            pltpu.VMEM((D, 6 * D), BF16),
            pltpu.VMEM((D, H * DH), BF16),
            pltpu.VMEM((H * DH, D), BF16),
            pltpu.VMEM((F, D), BF16),
            pltpu.VMEM((F, D), BF16),
            pltpu.VMEM((F, D), BF16),
            pltpu.VMEM((NG, B, T, DH), BF16),
            pltpu.VMEM((H, B, DH), BF16),
            pltpu.VMEM((B, D), F32),
            pltpu.VMEM((B, 4 * D), F32),
            pltpu.VMEM((B, D), BF16),
            pltpu.SemaphoreType.DMA((NG + 5 + D // DH + len(GU_CHUNKS) + len(D_CHUNKS),)),
        ],
        compiler_params=pltpu.CompilerParams(
            vmem_limit_bytes=64 * 1024 * 1024,
            disable_semaphore_checks=True,
        ),
    )(A_x.reshape(B, D), c, A_k_cache, A_v_cache, A_wq, A_wo,
      B_w_gate.T, B_w_up.T, B_w_down, w_mod)
    return out.reshape(B, 1, D)
```

```python
import jax
import jax.numpy as jnp
from jax import lax
import jax.experimental.pallas as pl
import jax.experimental.pallas.tpu as pltpu

F32 = jnp.float32
BF16 = jnp.bfloat16

T = 128
DEPTH = 13
STAG = 6
K_SHIFT = 64
ROWS = 32
GU_CHUNKS = (384, 384, 384, 224)
D_CHUNKS = (384, 384, 256, 352)
EPI = (8, 8, 8, 9)


def _chunks(sizes):
    out, r = [], 0
    for n in sizes:
        out.append((r, n))
        r += n
    return out


def _layernorm(x):
    m = jnp.mean(x, axis=-1, keepdims=True)
    xc = x - m
    v = jnp.mean(xc * xc, axis=-1, keepdims=True)
    return xc * lax.rsqrt(v + 1e-5)


def _mm(a, b):
    return jnp.dot(a, b, preferred_element_type=F32)


def _mm_t(a, b):
    return lax.dot_general(a, b, (((1,), (1,)), ((), ())), preferred_element_type=F32)


def _kernel(x_hbm, c_hbm, k_hbm, v_hbm, wq_hbm, wo_hbm, wg_hbm, wu_hbm, wd_hbm, wm_hbm, out_hbm,
            x_v, c_v, wm_v, wq_v, wo_v, wg_v, wu_v, wd_v, kv_v, q_v, acc_v, mod_v, out_v, sems):
    B, H, S, DH = k_hbm.shape
    F, D = wg_hbm.shape
    W = min(4096, max(256, S // 4))
    NK = W // T
    NG = 2 * NK
    NB = D // DH
    gu_ch, d_ch = _chunks(GU_CHUNKS), _chunks(D_CHUNKS)
    scale = DH ** -0.5

    kv_sem = lambda g: sems.at[g]
    c_sem, x_sem, wa_sem, wo_sem, wb_sem = (sems.at[NG + i] for i in range(5))
    q_sem = lambda j: sems.at[NG + 5 + j]
    gu_sem = lambda j: sems.at[NG + 5 + NB + j]
    d_sem = lambda j: sems.at[NG + 5 + NB + len(gu_ch) + j]

    queue = [0]

    def start(src, dst, sem):
        pltpu.make_async_copy(src, dst, sem).start(priority=queue[0])
        queue[0] ^= 1

    def start_list(copies):
        for src, dst, sl, sem in copies:
            start(src.at[sl], dst.at[sl], sem)

    def wait(dst, sem):
        pltpu.make_async_copy(dst, dst, sem).wait()

    pending = []

    def start_group(h, g):
        assert not (pending and g == 0)
        src, shift = (k_hbm, K_SHIFT) if g < NK else (v_hbm, 0)
        later = []
        for b in range(B):
            r = (g + 1 + STAG * b) % NK * T + shift
            n = min(T, W - r)
            start(src.at[b, h, pl.ds(S - W + r, n)], kv_v.at[g, b, pl.ds(0, n)], kv_sem(g))
            if n < T:
                later.append((src.at[b, h, pl.ds(S - W, T - n)], kv_v.at[g, b, pl.ds(n, T - n)], kv_sem(g)))
        for copy in pending:
            start(*copy)
        pending[:] = later

    def start_wq(j):
        for i in range(8):
            for c0 in range(0, H * DH, 2048):
                for half in range(2):
                    sl = (pl.ds(DH * j + 64 * half + 8 * i, 8), pl.ds(c0, 2048))
                    start(wq_hbm.at[sl], wq_v.at[sl], q_sem(j))

    wo_c = [(wo_hbm, wo_v, pl.ds(r + k * H * DH // 4, ROWS), wo_sem)
            for r in range(0, H * DH // 4, ROWS) for k in range(4)]
    wb_c = [(wm_hbm, wm_v, (pl.ds(r + k * D // 2, 8), pl.ds(2 * D, 4 * D)), wb_sem)
            for r in range(0, D // 2, 8) for k in range(2)]
    side = []
    for i in range(len(wb_c)):
        side += [wo_c[2 * i], wb_c[i], wo_c[2 * i + 1]]
    per = len(side) // NB

    late = []
    for j, (r, n) in enumerate(gu_ch):
        for i in range(0, n, ROWS):
            late.append((wg_hbm, wg_v, pl.ds(r + i, ROWS), gu_sem(j)))
            late.append((wu_hbm, wu_v, pl.ds(r + i, ROWS), gu_sem(j)))
    for j, (r, n) in enumerate(d_ch):
        for i in range(0, n, ROWS):
            late.append((wd_hbm, wd_v, pl.ds(r + i, ROWS), d_sem(j)))

    start(c_hbm, c_v, c_sem)
    start(x_hbm, x_v, x_sem)
    for r in [r0 + k * D // 4 for r0 in range(0, D // 4, 16) for k in range(4)]:
        sl = (pl.ds(r, 16), pl.ds(0, 2 * D))
        start(wm_hbm.at[sl], wm_v.at[sl], wa_sem)
    for j in range(NB - 1):
        start_wq(j)
    wait(c_v, c_sem)
    wait(x_v, x_sem)
    wait(wm_v.at[:, pl.ds(0, 2 * D)], wa_sem)
    start_wq(NB - 1)

    cv = c_v[...].astype(F32)
    silu_c = (cv * jax.nn.sigmoid(cv)).astype(BF16)
    mod_a = _mm(silu_c, wm_v[:, 0:2 * D])
    x = x_v[...].astype(F32)
    h1 = (_layernorm(x) * (1.0 + mod_a[:, D:2 * D]) + mod_a[:, 0:D]).astype(BF16)
    q = None
    for j in range(NB):
        wait(wq_v.at[pl.ds(DH * j, DH)], q_sem(j))
        start_list(side[j * per:(j + 1) * per])
        part = _mm(h1[:, DH * j:DH * (j + 1)], wq_v[pl.ds(DH * j, DH), :])
        q = part if q is None else q + part
    q = q.astype(BF16)
    for h in range(H):
        q_v[h] = q[:, h * DH:(h + 1) * DH]
    for g in range(DEPTH // 2):
        start_group(0, g)
    wait(wm_v.at[:, pl.ds(2 * D, 4 * D)], wb_sem)
    wait(wo_v, wo_sem)
    for g in range(DEPTH // 2, DEPTH):
        start_group(0, g)
    mod_v[...] = _mm(silu_c, wm_v[:, 2 * D:6 * D])
    acc_v[...] = jnp.zeros_like(acc_v)

    row = lax.broadcasted_iota(jnp.int32, (B, DH), 0)
    lane = lax.broadcasted_iota(jnp.int32, (B, T), 1)

    def own_rows(xs):
        r = xs[0]
        for b in range(1, B):
            r = jnp.where(row == b, xs[b], r)
        return r

    def head(h, issue):
        qh = q_v[h]
        s = []
        for g in range(NK):
            wait(kv_v.at[g], kv_sem(g))
            s.append(own_rows([_mm_t(qh, kv_v[g, b]) for b in range(B)]))
            issue(h, g)
        m = s[0]
        for t in s[1:]:
            m = jnp.maximum(m, t)
        m = jnp.max(m, axis=-1, keepdims=True)
        e = [jnp.exp((t - m) * scale) for t in s]
        l = e[0]
        for t in e[1:]:
            l = l + t
        l = jnp.sum(l, axis=-1, keepdims=True)
        if K_SHIFT:
            e = [pltpu.roll(t, K_SHIFT, 1) for t in e]
            e = [jnp.where(lane < K_SHIFT, e[g - 1], e[g]) for g in range(NK)]
        o = None
        for g in range(NK):
            wait(kv_v.at[NK + g], kv_sem(NK + g))
            p = e[g].astype(BF16)
            og = own_rows([_mm(p, kv_v[NK + g, b]) for b in range(B)])
            o = og if o is None else o + og
            issue(h, NK + g)
        acc_v[...] += _mm((o / l).astype(BF16), wo_v[pl.ds(pl.multiple_of(h * DH, DH), DH), :])

    def issue_steady(h, g):
        if g + DEPTH < NG:
            start_group(h, g + DEPTH)
        else:
            start_group(h + 1, g + DEPTH - NG)

    def issue_last(h, g):
        if g + DEPTH < NG:
            start_group(h, g + DEPTH)
        else:
            j = g + DEPTH - NG
            start_list(late[j * B:(j + 1) * B])

    def body(h, carry):
        head(h, issue_steady)
        return carry

    lax.fori_loop(0, H - 1, body, 0)
    head(H - 1, issue_last)

    rest = late[DEPTH * B:]
    pos = [0]

    def more(k):
        n = EPI[k] if k < len(EPI) else len(rest)
        start_list(rest[pos[0]:pos[0] + n])
        pos[0] += n

    ga, sb, cb, gb = (mod_v[:, i * D:(i + 1) * D] for i in range(4))
    more(0)
    x2 = x + ga * acc_v[...]
    h2 = (_layernorm(x2) * (1.0 + cb) + sb).astype(BF16)
    h3 = []
    for j, (r, n) in enumerate(gu_ch):
        wait(wg_v.at[pl.ds(r, n)], gu_sem(j))
        wait(wu_v.at[pl.ds(r, n)], gu_sem(j))
        more(j + 1)
        g = _mm_t(h2, wg_v[pl.ds(r, n), :])
        u = _mm_t(h2, wu_v[pl.ds(r, n), :])
        h3.append((jax.nn.sigmoid(g) * u).astype(BF16))
    more(len(EPI))
    h3 = jnp.concatenate(h3, axis=1)
    y = None
    for j, (r, n) in enumerate(d_ch):
        wait(wd_v.at[pl.ds(r, n)], d_sem(j))
        part = _mm(h3[:, r:r + n], wd_v[pl.ds(r, n), :])
        y = part if y is None else y + part
    out_v[...] = (x2 + gb * y).astype(BF16)
    done = pltpu.make_async_copy(out_v, out_hbm, c_sem)
    done.start()
    done.wait()


@jax.jit
def pallas_adaLN_cond__sliding_block_cached__glu_gated_glu__decode_kernel(
    A_x: jax.Array,
    A_k_cache: jax.Array,
    A_v_cache: jax.Array,
    A_wq: jax.Array,
    A_wo: jax.Array,
    B_x: jax.Array,
    B_w_gate: jax.Array,
    B_w_up: jax.Array,
    B_w_down: jax.Array,
    c: jax.Array,
    w_mod: jax.Array,
):
    del B_x
    B, _, D = A_x.shape
    _, H, S, DH = A_k_cache.shape
    F = B_w_gate.shape[1]
    W = min(4096, max(256, S // 4))
    NG = 2 * (W // T)
    assert (B, H, DH, D) == (8, 32, 128, 512) and W % T == 0 and F % ROWS == 0
    assert DEPTH <= NG and sum(GU_CHUNKS) == F == sum(D_CHUNKS)

    hbm = pl.BlockSpec(memory_space=pltpu.HBM)
    out = pl.pallas_call(
        _kernel,
        out_shape=jax.ShapeDtypeStruct((B, D), BF16),
        in_specs=[hbm] * 10,
        out_specs=hbm,
        scratch_shapes=[
            pltpu.VMEM((B, D), BF16),
            pltpu.VMEM((B, D), BF16),
            pltpu.VMEM((D, 6 * D), BF16),
            pltpu.VMEM((D, H * DH), BF16),
            pltpu.VMEM((H * DH, D), BF16),
            pltpu.VMEM((F, D), BF16),
            pltpu.VMEM((F, D), BF16),
            pltpu.VMEM((F, D), BF16),
            pltpu.VMEM((NG, B, T, DH), BF16),
            pltpu.VMEM((H, B, DH), BF16),
            pltpu.VMEM((B, D), F32),
            pltpu.VMEM((B, 4 * D), F32),
            pltpu.VMEM((B, D), BF16),
            pltpu.SemaphoreType.DMA((NG + 5 + D // DH + len(GU_CHUNKS) + len(D_CHUNKS),)),
        ],
        compiler_params=pltpu.CompilerParams(
            vmem_limit_bytes=64 * 1024 * 1024,
            disable_semaphore_checks=True,
        ),
    )(A_x.reshape(B, D), c, A_k_cache, A_v_cache, A_wq, A_wo,
      B_w_gate.T, B_w_up.T, B_w_down, w_mod)
    return out.reshape(B, 1, D)
```

```python
import jax
import jax.numpy as jnp
from jax import lax
import jax.experimental.pallas as pl
import jax.experimental.pallas.tpu as pltpu

F32 = jnp.float32
BF16 = jnp.bfloat16

T = 128
DEPTH = 13
STAG = 6
K_SHIFT = 64
ROWS = 32
GU_CHUNKS = (384, 384, 384, 224)
D_CHUNKS = (384, 384, 384, 224)
EPI = (8, 8, 8, 9)


def _chunks(sizes):
    out, r = [], 0
    for n in sizes:
        out.append((r, n))
        r += n
    return out


def _layernorm(x):
    m = jnp.mean(x, axis=-1, keepdims=True)
    xc = x - m
    v = jnp.mean(xc * xc, axis=-1, keepdims=True)
    return xc * lax.rsqrt(v + 1e-5)


def _mm(a, b):
    return jnp.dot(a, b, preferred_element_type=F32)


def _mm_t(a, b):
    return lax.dot_general(a, b, (((1,), (1,)), ((), ())), preferred_element_type=F32)


def _kernel(x_hbm, c_hbm, k_hbm, v_hbm, wq_hbm, wo_hbm, wg_hbm, wu_hbm, wd_hbm, wm_hbm, out_hbm,
            x_v, c_v, wm_v, wq_v, wo_v, wg_v, wu_v, wd_v, kv_v, q_v, acc_v, mod_v, out_v, sems):
    B, H, S, DH = k_hbm.shape
    F, D = wg_hbm.shape
    W = min(4096, max(256, S // 4))
    NK = W // T
    NG = 2 * NK
    NB = D // DH
    gu_ch, d_ch = _chunks(GU_CHUNKS), _chunks(D_CHUNKS)
    scale = DH ** -0.5

    kv_sem = lambda g: sems.at[g]
    c_sem, x_sem, wa_sem, wo_sem, wb_sem = (sems.at[NG + i] for i in range(5))
    q_sem = lambda j: sems.at[NG + 5 + j]
    gu_sem = lambda j: sems.at[NG + 5 + NB + j]
    d_sem = lambda j: sems.at[NG + 5 + NB + len(gu_ch) + j]

    queue = [0]

    def start(src, dst, sem):
        pltpu.make_async_copy(src, dst, sem).start(priority=queue[0])
        queue[0] ^= 1

    def start_list(copies):
        for copy in copies:
            start(*copy)

    def wait(dst, sem):
        pltpu.make_async_copy(dst, dst, sem).wait()

    pending = []

    def start_group(h, g):
        assert not (pending and g == 0)
        src, shift = (k_hbm, K_SHIFT) if g < NK else (v_hbm, 0)
        later = []
        for b in range(B):
            r = (g + 1 + STAG * b) % NK * T + shift
            n = min(T, W - r)
            start(src.at[b, h, pl.ds(S - W + r, n)], kv_v.at[g, b, pl.ds(0, n)], kv_sem(g))
            if n < T:
                later.append((src.at[b, h, pl.ds(S - W, T - n)], kv_v.at[g, b, pl.ds(n, T - n)], kv_sem(g)))
        start_list(pending)
        pending[:] = later

    def start_wq(j):
        for i in range(8):
            for c0 in range(0, H * DH, 2048):
                for half in range(2):
                    sl = (pl.ds(DH * j + 64 * half + 8 * i, 8), pl.ds(c0, 2048))
                    start(wq_hbm.at[sl], wq_v.at[sl], q_sem(j))

    same = lambda hbm, vmem, idx, sem: (hbm.at[idx], vmem.at[idx], sem)
    wo_c = [same(wo_hbm, wo_v, pl.ds(r + k * H * DH // 4, ROWS), wo_sem)
            for r in range(0, H * DH // 4, ROWS) for k in range(4)]
    wb_c = [same(wm_hbm, wm_v, (pl.ds(r + k * D // 2, 8), pl.ds(2 * D, 4 * D)), wb_sem)
            for r in range(0, D // 2, 8) for k in range(2)]
    side = []
    for i in range(len(wb_c)):
        side += [wo_c[2 * i], wb_c[i], wo_c[2 * i + 1]]
    per = len(side) // NB

    half = (F // ROWS + 1) // 2
    blocks = [i + k * half for i in range(half) for k in range(2)]

    def ffn_copy(hbm, vmem, r, sem):
        return hbm.at[pl.ds(blocks[r // ROWS] * ROWS, ROWS)], vmem.at[pl.ds(r, ROWS)], sem

    late = []
    for j, (r0, n) in enumerate(gu_ch):
        for r in range(r0, r0 + n, ROWS):
            late += [ffn_copy(wg_hbm, wg_v, r, gu_sem(j)), ffn_copy(wu_hbm, wu_v, r, gu_sem(j))]
    for j, (r0, n) in enumerate(d_ch):
        late += [ffn_copy(wd_hbm, wd_v, r, d_sem(j)) for r in range(r0, r0 + n, ROWS)]

    start(c_hbm, c_v, c_sem)
    start(x_hbm, x_v, x_sem)
    for r in [r0 + k * D // 4 for r0 in range(0, D // 4, 16) for k in range(4)]:
        sl = (pl.ds(r, 16), pl.ds(0, 2 * D))
        start(wm_hbm.at[sl], wm_v.at[sl], wa_sem)
    for j in range(NB - 1):
        start_wq(j)
    wait(c_v, c_sem)
    wait(x_v, x_sem)
    wait(wm_v.at[:, pl.ds(0, 2 * D)], wa_sem)
    start_wq(NB - 1)

    cv = c_v[...].astype(F32)
    silu_c = (cv * jax.nn.sigmoid(cv)).astype(BF16)
    mod_a = _mm(silu_c, wm_v[:, 0:2 * D])
    x = x_v[...].astype(F32)
    h1 = (_layernorm(x) * (1.0 + mod_a[:, D:2 * D]) + mod_a[:, 0:D]).astype(BF16)
    q = None
    for j in range(NB):
        wait(wq_v.at[pl.ds(DH * j, DH)], q_sem(j))
        start_list(side[j * per:(j + 1) * per])
        part = _mm(h1[:, DH * j:DH * (j + 1)], wq_v[pl.ds(DH * j, DH), :])
        q = part if q is None else q + part
    q = q.astype(BF16)
    for h in range(H):
        q_v[h] = q[:, h * DH:(h + 1) * DH]
    for g in range(DEPTH // 2):
        start_group(0, g)
    wait(wm_v.at[:, pl.ds(2 * D, 4 * D)], wb_sem)
    wait(wo_v, wo_sem)
    for g in range(DEPTH // 2, DEPTH):
        start_group(0, g)
    mod_v[...] = _mm(silu_c, wm_v[:, 2 * D:6 * D])
    acc_v[...] = jnp.zeros_like(acc_v)

    row = lax.broadcasted_iota(jnp.int32, (B, DH), 0)
    lane = lax.broadcasted_iota(jnp.int32, (B, T), 1)

    def own_rows(xs):
        r = xs[0]
        for b in range(1, B):
            r = jnp.where(row == b, xs[b], r)
        return r

    def head(h, issue):
        qh = q_v[h]
        s = []
        for g in range(NK):
            wait(kv_v.at[g], kv_sem(g))
            s.append(own_rows([_mm_t(qh, kv_v[g, b]) for b in range(B)]))
            issue(h, g)
        m = s[0]
        for t in s[1:]:
            m = jnp.maximum(m, t)
        m = jnp.max(m, axis=-1, keepdims=True)
        e = [jnp.exp((t - m) * scale) for t in s]
        l = e[0]
        for t in e[1:]:
            l = l + t
        l = jnp.sum(l, axis=-1, keepdims=True)
        if K_SHIFT:
            e = [pltpu.roll(t, K_SHIFT, 1) for t in e]
            e = [jnp.where(lane < K_SHIFT, e[g - 1], e[g]) for g in range(NK)]
        o = None
        for g in range(NK):
            wait(kv_v.at[NK + g], kv_sem(NK + g))
            p = e[g].astype(BF16)
            og = own_rows([_mm(p, kv_v[NK + g, b]) for b in range(B)])
            o = og if o is None else o + og
            issue(h, NK + g)
        acc_v[...] += _mm((o / l).astype(BF16), wo_v[pl.ds(pl.multiple_of(h * DH, DH), DH), :])

    def issue_steady(h, g):
        if g + DEPTH < NG:
            start_group(h, g + DEPTH)
        else:
            start_group(h + 1, g + DEPTH - NG)

    def issue_last(h, g):
        if g + DEPTH < NG:
            start_group(h, g + DEPTH)
        else:
            j = g + DEPTH - NG
            start_list(late[j * B:(j + 1) * B])

    def body(h, carry):
        head(h, issue_steady)
        return carry

    lax.fori_loop(0, H - 1, body, 0)
    head(H - 1, issue_last)

    rest = late[DEPTH * B:]
    pos = [0]

    def more(k):
        n = EPI[k] if k < len(EPI) else len(rest)
        start_list(rest[pos[0]:pos[0] + n])
        pos[0] += n

    ga, sb, cb, gb = (mod_v[:, i * D:(i + 1) * D] for i in range(4))
    more(0)
    x2 = x + ga * acc_v[...]
    h2 = (_layernorm(x2) * (1.0 + cb) + sb).astype(BF16)
    h3 = []
    for j, (r, n) in enumerate(gu_ch):
        wait(wg_v.at[pl.ds(r, n)], gu_sem(j))
        wait(wu_v.at[pl.ds(r, n)], gu_sem(j))
        more(j + 1)
        g = _mm_t(h2, wg_v[pl.ds(r, n), :])
        u = _mm_t(h2, wu_v[pl.ds(r, n), :])
        h3.append((jax.nn.sigmoid(g) * u).astype(BF16))
    more(len(EPI))
    h3 = jnp.concatenate(h3, axis=1)
    y = None
    for j, (r, n) in enumerate(d_ch):
        wait(wd_v.at[pl.ds(r, n)], d_sem(j))
        part = _mm(h3[:, r:r + n], wd_v[pl.ds(r, n), :])
        y = part if y is None else y + part
    out_v[...] = (x2 + gb * y).astype(BF16)
    done = pltpu.make_async_copy(out_v, out_hbm, c_sem)
    done.start()
    done.wait()


@jax.jit
def pallas_adaLN_cond__sliding_block_cached__glu_gated_glu__decode_kernel(
    A_x: jax.Array,
    A_k_cache: jax.Array,
    A_v_cache: jax.Array,
    A_wq: jax.Array,
    A_wo: jax.Array,
    B_x: jax.Array,
    B_w_gate: jax.Array,
    B_w_up: jax.Array,
    B_w_down: jax.Array,
    c: jax.Array,
    w_mod: jax.Array,
):
    del B_x
    B, _, D = A_x.shape
    _, H, S, DH = A_k_cache.shape
    F = B_w_gate.shape[1]
    W = min(4096, max(256, S // 4))
    NG = 2 * (W // T)
    assert (B, H, DH, D) == (8, 32, 128, 512) and W % T == 0 and F % ROWS == 0
    assert DEPTH <= NG and sum(GU_CHUNKS) == F == sum(D_CHUNKS)

    hbm = pl.BlockSpec(memory_space=pltpu.HBM)
    out = pl.pallas_call(
        _kernel,
        out_shape=jax.ShapeDtypeStruct((B, D), BF16),
        in_specs=[hbm] * 10,
        out_specs=hbm,
        scratch_shapes=[
            pltpu.VMEM((B, D), BF16),
            pltpu.VMEM((B, D), BF16),
            pltpu.VMEM((D, 6 * D), BF16),
            pltpu.VMEM((D, H * DH), BF16),
            pltpu.VMEM((H * DH, D), BF16),
            pltpu.VMEM((F, D), BF16),
            pltpu.VMEM((F, D), BF16),
            pltpu.VMEM((F, D), BF16),
            pltpu.VMEM((NG, B, T, DH), BF16),
            pltpu.VMEM((H, B, DH), BF16),
            pltpu.VMEM((B, D), F32),
            pltpu.VMEM((B, 4 * D), F32),
            pltpu.VMEM((B, D), BF16),
            pltpu.SemaphoreType.DMA((NG + 5 + D // DH + len(GU_CHUNKS) + len(D_CHUNKS),)),
        ],
        compiler_params=pltpu.CompilerParams(
            vmem_limit_bytes=64 * 1024 * 1024,
            disable_semaphore_checks=True,
        ),
    )(A_x.reshape(B, D), c, A_k_cache, A_v_cache, A_wq, A_wo,
      B_w_gate.T, B_w_up.T, B_w_down, w_mod)
    return out.reshape(B, 1, D)
```
